```python
import os as _os
_os.environ.setdefault("JAX_PLATFORMS", "cpu")
import jax
import jax.numpy as jnp

def _softmax(x, axis=-1):
    return jax.nn.softmax(x, axis=axis)
def _gelu(x):
    return jax.nn.gelu(x, approximate=True)
def _silu(x):
    return jax.nn.silu(x)
def _sigmoid(x):
    return jax.nn.sigmoid(x)
def _layernorm(x, axis=-1, eps=1e-5):
    m = jnp.mean(x, axis=axis, keepdims=True)
    v = jnp.var(x, axis=axis, keepdims=True)
    return (x - m) / jnp.sqrt(v + eps)
def _scatter_add(tgt, idx, src, axis=0):
    return tgt.at[idx].add(src)
def _segment_sum(src, seg, n):
    return jax.ops.segment_sum(src, seg, n)
class _Rng:
    def __init__(self, key):
        self._k = key
    def _next(self):
        self._k, sub = jax.random.split(self._k)
        return sub
    def normal(self, shape):
        return jax.random.normal(self._next(), shape, dtype=jnp.bfloat16)
    def randint(self, lo, hi, shape):
        return jax.random.randint(self._next(), shape, lo, hi, dtype=jnp.int32)
    def uniform(self, shape, lo=0.0, hi=1.0):
        return jax.random.uniform(self._next(), shape, jnp.bfloat16, lo, hi)
    def permutation(self, n):
        return jax.random.permutation(self._next(), n)


kernel_name = 'concat_heads__mha_block_cached__mha_block_cached__near_ridge'

def setup_inputs():
    _rng = _Rng(jax.random.key(int.from_bytes(__import__("os").urandom(4), "little")))
    _w = (lambda a: (lambda t: t.astype(jnp.bfloat16) if jnp.issubdtype(t.dtype, jnp.floating) else t)(jnp.asarray(a)))
    def _A_setup():
        B, Sq, D = 16, 32, 1024
        H, Sk, Dh = 32, 32, 128
        return {
            "x": _w((lambda *s: _rng.normal(s) * 0.8)(B, Sq, D)),
            "k_cache": _w((lambda *s: _rng.normal(s) * 0.8)(B, H, Sk, Dh)),
            "v_cache": _w((lambda *s: _rng.normal(s) * 0.05)(B, H, Sk, Dh)),
            "wq": _w((lambda *s: _rng.normal(s) * 0.8)(D, H * Dh) * (D ** -0.5)),
            "wo": _w((lambda *s: _rng.normal(s) * 0.05)(H * Dh, D) * ((H * Dh) ** -0.5)),
        }
    _A_in = _A_setup()

    def _B_setup():
        B, Sq, D = 16, 32, 1024
        H, Sk, Dh = 32, 32, 128
        return {
            "x": _w((lambda *s: _rng.normal(s) * 0.8)(B, Sq, D)),
            "k_cache": _w((lambda *s: _rng.normal(s) * 0.8)(B, H, Sk, Dh)),
            "v_cache": _w((lambda *s: _rng.normal(s) * 0.05)(B, H, Sk, Dh)),
            "wq": _w((lambda *s: _rng.normal(s) * 0.8)(D, H * Dh) * (D ** -0.5)),
            "wo": _w((lambda *s: _rng.normal(s) * 0.05)(H * Dh, D) * ((H * Dh) ** -0.5)),
        }
    _B_in = _B_setup()

    return {
        "A_x": _A_in["x"],
        "A_k_cache": _A_in["k_cache"],
        "A_v_cache": _A_in["v_cache"],
        "A_wq": _A_in["wq"],
        "A_wo": _A_in["wo"],
        "B_x": _B_in["x"],
        "B_k_cache": _B_in["k_cache"],
        "B_v_cache": _B_in["v_cache"],
        "B_wq": _B_in["wq"],
        "B_wo": _B_in["wo"],
    }

def reference(A_x, A_k_cache, A_v_cache, A_wq, A_wo, B_x, B_k_cache, B_v_cache, B_wq, B_wo):
    def _A_ref(x, k_cache, v_cache, wq, wo):
        B, Sq, D = x.shape
        H, Dh = 32, 128
        q = (lambda x, *d: x.transpose(*d))((x @ wq).reshape(B, Sq, H, Dh), 0, 2, 1, 3)
        scores = jnp.einsum("bhqd,bhkd->bhqk", q, k_cache) * (Dh ** -0.5)
        p = _softmax(scores, axis=-1)
        o = jnp.einsum("bhqk,bhkd->bhqd", p, v_cache)
        return (lambda x, *d: x.transpose(*d))(o, 0, 2, 1, 3).reshape(B, Sq, H * Dh) @ wo

    def _B_ref(x, k_cache, v_cache, wq, wo):
        B, Sq, D = x.shape
        H, Dh = 32, 128
        q = (lambda x, *d: x.transpose(*d))((x @ wq).reshape(B, Sq, H, Dh), 0, 2, 1, 3)
        scores = jnp.einsum("bhqd,bhkd->bhqk", q, k_cache) * (Dh ** -0.5)
        p = _softmax(scores, axis=-1)
        o = jnp.einsum("bhqk,bhkd->bhqd", p, v_cache)
        return (lambda x, *d: x.transpose(*d))(o, 0, 2, 1, 3).reshape(B, Sq, H * Dh) @ wo

    a = _A_ref(A_x, A_k_cache, A_v_cache, A_wq, A_wo)
    b = _B_ref(B_x, B_k_cache, B_v_cache, B_wq, B_wo)
    return jnp.concatenate([a, b], axis=-1)
```

```python
import functools
import math
import jax
import jax.numpy as jnp
from jax import lax
import jax.experimental.pallas as pl
import jax.experimental.pallas.tpu as pltpu

B, SQ, D = 16, 32, 1024
H, SK, DH = 32, 32, 128
M = B * SQ
T = 128
F32, BF16, U32 = jnp.float32, jnp.bfloat16, jnp.uint32

ALPHA = [((0, 0, 1), (1, 1, 1)), ((1, 0, 1), (1, 1, 1)), ((0, 0, 1),), ((1, 1, 1),),
         ((0, 0, 1), (0, 1, 1)), ((1, 0, 1), (0, 0, -1)), ((0, 1, 1), (1, 1, -1))]
BETA = [((0, 0, 1), (1, 1, 1)), ((0, 0, 1),), ((0, 1, 1), (1, 1, -1)), ((1, 0, 1), (0, 0, -1)),
        ((1, 1, 1),), ((0, 0, 1), (0, 1, 1)), ((1, 0, 1), (1, 1, 1))]
GAMMA = [((0, 0, 1), (1, 1, 1)), ((1, 0, 1), (1, 1, -1)), ((0, 1, 1), (1, 1, 1)), ((0, 0, 1), (1, 0, 1)),
         ((0, 1, 1), (0, 0, -1)), ((1, 1, 1),), ((0, 0, 1),)]


def lincomb(terms, get):
    terms = sorted(terms, key=lambda t: -t[2])
    assert terms[0][2] > 0
    v = get(*terms[0][:2])
    for i, j, s in terms[1:]:
        v = v + get(i, j) if s > 0 else v - get(i, j)
    return v


class Fold:
    def __init__(self, order):
        self.left = {}
        for a in order:
            for i, k, _ in GAMMA[a]:
                self.left[i, k] = self.left.get((i, k), 0) + 1
        self.acc = {}

    def add(self, a, m):
        done = []
        for i, k, s in GAMMA[a]:
            if (i, k) not in self.acc:
                self.acc[i, k] = (s, m)
            else:
                s0, c = self.acc[i, k]
                if s0 > 0:
                    c = [x + y if s > 0 else x - y for x, y in zip(c, m)]
                elif s > 0:
                    c = [y - x for x, y in zip(c, m)]
                else:
                    c = [x + y for x, y in zip(c, m)]
                self.acc[i, k] = (-1 if (s0 < 0 and s < 0) else 1, c)
            self.left[i, k] -= 1
            if self.left[i, k] == 0:
                s0, c = self.acc.pop((i, k))
                assert s0 > 0
                done.append((i, k, c))
        return done


class Schedule:
    def __init__(self):
        self.items = []

    def spread(self, tasks, start, end):
        for k, t in enumerate(tasks):
            self.items.append((start + (end - start) * (k + 0.5) / len(tasks), len(self.items), t))

    def run_until(self, pos):
        self.items.sort(key=lambda it: it[:2])
        while self.items and self.items[0][0] <= pos:
            self.items.pop(0)[2]()


def make(flags=None, q_outer=(1, 3, 0, 5, 2, 4, 6), o_outer=(1, 0, 2, 4, 3, 5, 6),
         inner=(1, 4, 0, 5, 2, 3, 6), lead=7, olead=7, fine=True, nodma=False,
         n1=3, xbg=False, arange=(0, 49), fuse_last=True, ostage=False, last_outer=(0, 1, 2, 3, 4, 5, 6), chunk=64, narrow=True, accn=False, pad=0, dq=False, do=False, midwait=True, nosem=False, nobound=False):
    G = 4
    GA = 8
    NG = 2 * H // G
    NA = 2 * H // GA
    P = 49
    c_exp = (DH ** -0.5) * math.log2(math.e)

    def first_use(coef, outer):
        seen, per = [], []
        for a in outer:
            new = [(i, j) for i, j, _ in coef[a] if (i, j) not in seen]
            seen += new
            per.append(new)
        return dict(zip(outer, per))

    def kernel(ax, ak, av, awq, awo, bx, bk, bv, bwq, bwo, out_hbm,
               x_buf, wq_buf, k_buf, v_buf, wo_buf,
               xp, wqs, wos, q_buf, o_even, o_odd, os_, acc, out_buf,
               in_sem, out_sem):
        XQ, XB, WQ0, K0, V0, WO0 = 0, 4, 5, 5 + 4 * NG, 5 + 4 * NG + NA, 5 + 4 * NG + 2 * NA
        k32, v32 = k_buf.bitcast(U32), v_buf.bitcast(U32)
        scope = jax.named_scope

        def quad(ref, i, j):
            r, c = ref.shape[0] // 2, ref.shape[1] // 2
            return ref.at[pl.ds(i * r, r), pl.ds(j * c, c)]

        def start(src, dst, sem):
            if not nodma:
                pltpu.make_async_copy(src, dst, in_sem.at[sem]).start()

        def wait_for(dst, sem):
            if not nodma:
                pltpu.make_async_copy(dst, dst, in_sem.at[sem]).wait()

        def shuffle_lanes(w):
            lane = lax.broadcasted_iota(jnp.int32, w.shape, 1)
            return jnp.take_along_axis(w, (lane & ~15) | ((lane & 15) >> 1) | ((lane & 1) << 3), axis=1)

        def pack(w):
            return pltpu.pack_elementwise([w[:8], w[8:]], packed_dtype=BF16)

        def x_tasks(blk, outers):
            def task(r, c):
                @functools.cache
                def patch(i, j):
                    w = pltpu.bitcast(x_buf[blk, pl.ds(i * T + r * 16, 16), pl.ds(j * 256 + c * T, T)], U32)
                    return jnp.concatenate([pltpu.unpack_elementwise(w, index=h, packed_dtype=BF16, unpacked_dtype=F32)
                                            for h in range(2)], axis=0)
                for a in outers:
                    v = [[lincomb(ALPHA[a], lambda i, j: patch(2 * i + i2, 2 * j + j2)) for j2 in range(2)]
                         for i2 in range(2)]
                    for b in inner:
                        xp[blk, 7 * a + b, c, pl.ds(r * 8, 8), :] = pack(lincomb(ALPHA[b], lambda i, j: v[i][j]))
            return [functools.partial(task, r, c) for r in range(T // 16) for c in range(2)]

        class Stage:
            def __init__(self, src, dst, a, slot, z):
                self.src, self.dst, self.a, self.slot = src, dst, a, slot
                self.br, self.bc = src.shape[0] // 4, src.shape[1] // 4
                self.before = None

            def direct(self):
                return len(BETA[self.a]) == 1 and (dq if self.bc == T else do)

            def tasks(self):
                if self.direct():
                    return []
                br, bc = self.br, self.bc
                rows = chunk * T // bc

                def task(r0):
                    v = lincomb(
                        BETA[self.a], lambda j, k: self.src[pl.ds(2 * j * br + r0, rows), pl.ds(2 * k * bc, 2 * bc)].astype(F32))
                    if narrow:
                        for c in range(2 * bc // T):
                            self.dst[self.slot, c, pl.ds(r0 + (r0 // br) * pad, rows), :] = v[:, c * T:(c + 1) * T]
                    else:
                        self.dst[self.slot, pl.ds(r0, rows), :] = v
                return [functools.partial(task, r0) for r0 in range(0, 2 * br, rows)]

            def rhs(self, b):
                br, bc = self.br, self.bc
                if self.direct():
                    j1, k1, _ = BETA[self.a][0]
                    return lincomb(BETA[b], lambda j, k: self.src[pl.ds((2 * j1 + j) * br, br),
                                                                  pl.ds((2 * k1 + k) * bc, bc)].astype(F32)).astype(BF16)
                if narrow:
                    n = bc // T
                    return jnp.concatenate(
                        [lincomb(BETA[b], lambda j, k: self.dst[self.slot, k * n + c, pl.ds(j * (br + pad), br), :]) for c in range(n)],
                        axis=1).astype(BF16)
                return lincomb(BETA[b], lambda j, k: self.dst[self.slot, pl.ds(j * br, br), pl.ds(k * bc, bc)]).astype(BF16)

        lane_grp = lax.broadcasted_iota(jnp.int32, (SK, T), 1) // SQ

        def attn_tasks(t, o_ref):
            tiles = [(hh, j) for hh in range(GA) for j in range(4)]
            state = {}

            def s1(hh, j):
                kt = pltpu.bitcast(k32[t, pl.ds(4 * j, 4), hh].reshape(T // 2, DH), BF16)
                qt = q_buf[2 * t + hh // G, pl.ds(j * T, T), pl.ds(hh % G * DH, DH)]
                st = lax.dot_general(kt, qt, (((1,), (1,)), ((), ())), preferred_element_type=F32)
                s = st[0:SK]
                for b in range(1, 4):
                    s = jnp.where(lane_grp == b, st[b * SK:(b + 1) * SK], s)
                state[hh, j] = s

            def s2(hh, j):
                s = state[hh, j]
                e = jnp.exp2((s - jnp.max(s, axis=0, keepdims=True)) * c_exp)
                p = e * (1.0 / jnp.sum(e, axis=0, keepdims=True))
                pt = jnp.concatenate([jnp.where(lane_grp == b, p, 0.0) for b in range(4)], axis=0)
                state[hh, j] = pt.astype(BF16).T

            def s3(hh, j):
                vt = pltpu.bitcast(v32[t, pl.ds(4 * j, 4), hh].reshape(T // 2, DH), BF16)
                o_ref[hh, pl.ds(j * T, T), :] = jnp.dot(state.pop((hh, j)), vt, preferred_element_type=F32)

            tasks = []
            nt = len(tiles)
            for i in range(nt + 2):
                if i < nt:
                    tasks.append(functools.partial(s1, *tiles[i]))
                if 1 <= i <= nt:
                    tasks.append(functools.partial(s2, *tiles[i - 1]))
                if i >= 2:
                    tasks.append(functools.partial(s3, *tiles[i - 2]))
            return tasks

        def run_products(product, outer, stages, sched, base=0, emit=None, lead=lead):
            top = {key: Fold(outer) for key in ((0, 0), (0, 1), (1, 0), (1, 1))}
            for n, a in enumerate(outer):
                if n + 1 < len(stages):
                    if stages[n + 1].before:
                        stages[n + 1].before()
                    sched.spread(stages[n + 1].tasks(), base + 7 * n, base + 7 * n + lead)
                sub = Fold(inner)
                for s, b in enumerate(inner):
                    m = product(a, b, stages[n].rhs(b))
                    sched.run_until(base + 7 * n + s + 1)
                    if emit is not None:
                        for i2, k2, c2 in sub.add(b, [m]):
                            for i1, k1, c1 in top[i2, k2].add(a, c2):
                                emit(2 * i1 + i2, 2 * k1 + k2, c1[0])

        def q_phase(g, stages, sched, base=0):
            def product(a, b, rhs):
                lhs = jnp.concatenate([pltpu.bitcast(xp[g // 8, 7 * a + b, c], BF16) for c in range(2)], axis=1)
                return jnp.dot(lhs, rhs, preferred_element_type=F32)

            def emit(i, k, v):
                q_buf[g, pl.ds(i * T, T), pl.ds(k * DH, DH)] = v.astype(BF16)
            run_products(product, q_outer, stages, sched, base, emit)

        def out_copy(blk, r0, nr, c0, nc):
            return pltpu.make_async_copy(out_buf.at[blk, pl.ds(r0, nr), pl.ds(c0, nc)],
                                         out_hbm.at[pl.ds(r0, nr), pl.ds(blk * D + c0, nc)], out_sem.at[blk])

        def acc_get(p, rows=slice(None)):
            if accn:
                return jnp.concatenate([acc[p, c, rows, :] for c in range(2)], axis=1)
            return acc[p, rows, :]

        class OStage:
            def __init__(self, o_ref, a, slot):
                self.o_ref, self.a, self.slot = o_ref, a, slot

            def tasks(self):
                if len(ALPHA[self.a]) == 1:
                    return []

                def task(h, i2):
                    os_[self.slot, h, pl.ds(i2 * T, T), :] = lincomb(
                        ALPHA[self.a], lambda i, j: self.o_ref[4 * j + h, pl.ds((2 * i + i2) * T, T), :])
                return [functools.partial(task, h, i2) for h in range(4) for i2 in range(2)]

            def block(self, i2, j2, c):
                if len(ALPHA[self.a]) == 1:
                    i, j, _ = ALPHA[self.a][0]
                    return self.o_ref[4 * j + 2 * j2 + c, pl.ds((2 * i + i2) * T, T), :]
                return os_[self.slot, 2 * j2 + c, pl.ds(i2 * T, T), :]

        def o_phase(first, o_ref, outer, stages, sched, final_blk=None):
            ost = {a: OStage(o_ref, a, n % 2) for n, a in enumerate(outer)}
            if ostage:
                for task in ost[outer[0]].tasks():
                    task()
                for n, a in enumerate(outer[1:]):
                    if ost[a].tasks():
                        sched.spread(ost[a].tasks(), 7 * n, 7 * n + olead)

            def raw(a, b, rhs):
                if ostage:
                    cols = [lincomb(ALPHA[b], lambda i, j: ost[a].block(i, j, c)) for c in range(2)]
                else:
                    terms = [(2 * i1 + i2, 2 * j1 + j2, s1 * s2) for i1, j1, s1 in ALPHA[a] for i2, j2, s2 in ALPHA[b]]
                    cols = [lincomb(terms, lambda i, j: o_ref[2 * j + c, pl.ds(i * T, T), :]) for c in range(2)]
                return jnp.dot(jnp.concatenate(cols, axis=1).astype(BF16), rhs, preferred_element_type=F32)

            if final_blk is None:
                def product(a, b, rhs):
                    prev = acc_get(7 * a + b)
                    new = (prev if first is None else jnp.where(first, 0.0, prev)) + raw(a, b, rhs)
                    if accn:
                        for c in range(2):
                            acc[7 * a + b, c] = new[:, c * T:(c + 1) * T]
                    else:
                        acc[7 * a + b] = new
                run_products(product, outer, stages, sched, lead=olead)
            else:
                def emit(i, k, v):
                    out_buf[final_blk, pl.ds(i * T, T), pl.ds(k * 256, 256)] = v.astype(BF16)
                    out_copy(final_blk, i * T, T, k * 256, 256).start()
                run_products(lambda a, b, rhs: raw(a, b, rhs) + acc_get(7 * a + b), outer, stages, sched, 0, emit, lead=olead)

        def finalize(blk):
            for r in range(T // 8):
                top = Fold(range(7))
                for a in range(7):
                    sub = Fold(range(7))
                    res = {}
                    for b in range(7):
                        for i, k, c in sub.add(b, [acc_get(7 * a + b, pl.ds(r * 8, 8))]):
                            res[i, k] = c[0]
                    keys = sorted(res)
                    for i1, k1, cs in top.add(a, [res[key] for key in keys]):
                        for (i2, k2), c in zip(keys, cs):
                            out_buf[blk, pl.ds((2 * i1 + i2) * T + r * 8, 8), pl.ds((2 * k1 + k2) * 256, 256)] = c.astype(BF16)
                if r % 4 == 3:
                    for i in range(4):
                        out_copy(blk, i * T + (r - 3) * 8, 32, 0, D).start()

        x_new, wq_new, wo_new = first_use(ALPHA, q_outer), first_use(BETA, q_outer), first_use(BETA, o_outer)
        wq_head = wq_new[q_outer[0]]
        wq_rest = [ij for a in q_outer[1:] for ij in wq_new[a]]

        def wq_start(g, quads):
            src = (awq, bwq)[g // 8].at[:, pl.ds((g % 8) * G * DH, G * DH)]
            for i, j in quads:
                start(quad(src, i, j), quad(wq_buf.at[g], i, j), WQ0 + 4 * g + 2 * i + j)

        def wq_wait(g, quads):
            for i, j in quads:
                wait_for(quad(wq_buf.at[g], i, j), WQ0 + 4 * g + 2 * i + j)

        def step_start(t):
            heads = pl.ds((t % 4) * GA, GA)
            start((ak, bk)[t // 4].at[:, heads], k_buf.at[t], K0 + t)
            start((av, bv)[t // 4].at[:, heads], v_buf.at[t], V0 + t)
            start((awo, bwo)[t // 4].at[pl.ds((t % 4) * GA * DH, GA * DH), :], wo_buf.at[t], WO0 + t)

        def step_wait(t):
            wait_for(k_buf.at[t], K0 + t)
            wait_for(v_buf.at[t], V0 + t)
            wait_for(wo_buf.at[t], WO0 + t)

        for a in q_outer:
            for i, j in x_new[a]:
                start(quad(ax, i, j), quad(x_buf.at[0], i, j), XQ + 2 * i + j)
            wq_start(0, wq_new[a])
        NF = 2 + n1
        for g in range(1, NG):
            if g < NF:
                wq_start(g, wq_head)
                wq_start(g, wq_rest)
            else:
                start((awq, bwq)[g // 8].at[:, pl.ds((g % 8) * G * DH, G * DH)], wq_buf.at[g], WQ0 + 4 * g)
            if g == 8:
                start(bx, x_buf.at[1], XB)
        for t in range(NA):
            step_start(t)

        def stages_of(src, dst, outer, z):
            return [Stage(src, dst, a, 0 if n == 0 else 1 + (n - 1) % 2, z) for n, a in enumerate(outer)]

        wq_stages = lambda g, z=0: stages_of(wq_buf.at[g], wqs, q_outer, 0)
        wo_stages = lambda t, outer=o_outer: stages_of(wo_buf.at[t], wos, outer, 0)

        with scope("S_q0"):
            def arrive(outers):
                for a in outers:
                    for i, j in x_new[a]:
                        wait_for(quad(x_buf.at[0], i, j), XQ + 2 * i + j)
                    wq_wait(0, wq_new[a])
                for task in x_tasks(0, outers):
                    task()

            st = wq_stages(0) + wq_stages(1)[:1]
            cuts = fine if isinstance(fine, tuple) else (tuple(range(8)) if fine else (0, 7))
            for lo, hi in zip(cuts, cuts[1:]):
                st[lo].before = functools.partial(arrive, q_outer[lo:hi])
            st[7].before = lambda: wq_wait(1, wq_head)
            st[0].before()
            for task in st[0].tasks():
                task()
            q_phase(0, st, Schedule())

        def q_groups(g0, n, sched):
            if n == 1:
                wq_wait(g0, wq_rest)
                wq_wait(g0 + 1, wq_head)
            else:
                for d in range(n):
                    wait_for(wq_buf.at[g0 + d + 1], WQ0 + 4 * (g0 + d + 1))
            for d in range(n):
                q_phase(g0 + d, wq_stages(g0 + d, g0 >> 5) + wq_stages(g0 + d + 1, g0 >> 5)[:1], sched, d * P)

        @pl.loop(1, 1 + n1)
        def _(g):
            with scope("S_q1"):
                q_groups(g, 1, Schedule())

        wq_wait(NF - 1, wq_rest)
        if xbg:
            assert n1 == 5
            with scope("S_qx"):
                wait_for(x_buf.at[1], XB)
                sched = Schedule()
                sched.spread(x_tasks(1, q_outer), 0, 2 * P)
                q_groups(6, 2, sched)

        @pl.loop(8 if xbg else 1 + n1, NG - 2, step=2)
        def _(g0):
            with scope("S_q2"):
                if not xbg:
                    @pl.when(g0 == 8)
                    def _():
                        wait_for(x_buf.at[1], XB)
                        for task in x_tasks(1, q_outer):
                            task()
                q_groups(g0, 2, Schedule())

        with scope("S_qa"):
            wait_for(wq_buf.at[NG - 1], WQ0 + 4 * (NG - 1))
            step_wait(0)
            sched = Schedule()
            sched.spread(attn_tasks(0, o_even), 0, 2 * P)
            q_phase(NG - 2, wq_stages(NG - 2) + wq_stages(NG - 1)[:1], sched)
            q_phase(NG - 1, wq_stages(NG - 1) + wo_stages(0)[:1], sched, P)

        def ao_phase(t, first, cur, nxt, next_outer=o_outer):
            sched = Schedule()
            sched.spread(attn_tasks(t + 1, nxt), *arange)
            o_phase(first, cur, o_outer, wo_stages(t) + wo_stages(t + 1, next_outer)[:1], sched)

        @pl.loop(0, NA - 2, step=2)
        def _(t):
            with scope("S_ao"):
                step_wait(t + 1)
                if not midwait:
                    step_wait(t + 2)
                ao_phase(t, t % 4 == 0, o_even, o_odd)
                if midwait:
                    step_wait(t + 2)
                ao_phase(t + 1, None, o_odd, o_even)

                @pl.when(t == 2)
                def _():
                    finalize(0)

        with scope("S_last"):
            step_wait(NA - 1)
            ao_phase(NA - 2, None, o_even, o_odd, last_outer)
            o_phase(None, o_odd, last_outer, wo_stages(NA - 1, last_outer), Schedule(), 1 if fuse_last else None)
        pltpu.make_async_copy(out_buf.at[0], out_buf.at[0], out_sem.at[0]).wait()
        if not fuse_last:
            with scope("S_fin"):
                finalize(1)
        pltpu.make_async_copy(out_buf.at[1], out_buf.at[1], out_sem.at[1]).wait()

    def fn(A_x, A_k, A_v, A_wq, A_wo, B_x, B_k, B_v, B_wq, B_wo):
        any_spec = pl.BlockSpec(memory_space=pl.ANY)
        out = pl.pallas_call(
            kernel,
            in_specs=[any_spec] * 10,
            out_specs=any_spec,
            out_shape=jax.ShapeDtypeStruct((M, 2 * D), BF16),
            scratch_shapes=[
                pltpu.VMEM((2, M, D), BF16),
                pltpu.VMEM((NG, D, G * DH), BF16),
                pltpu.VMEM((NA, B, GA, SK, DH), BF16),
                pltpu.VMEM((NA, B, GA, SK, DH), BF16),
                pltpu.VMEM((NA, GA * DH, D), BF16),
                pltpu.VMEM((2, P, 2, T // 2, T), U32),
                pltpu.VMEM((3, 2, 512 + 2 * pad, T) if narrow else (3, 512, 256), F32),
                pltpu.VMEM((3, 4, 512 + 2 * pad, T) if narrow else (3, 512, 512), F32),
                pltpu.VMEM((NG, M, G * DH), BF16),
                pltpu.VMEM((GA, M, DH), F32),
                pltpu.VMEM((GA, M, DH), F32),
                pltpu.VMEM((2, 4, 2 * T, T), F32),
                pltpu.VMEM((P, 2, T, T) if accn else (P, T, 256), F32),
                pltpu.VMEM((2, M, D), BF16),
                pltpu.SemaphoreType.DMA((5 + 4 * NG + 3 * NA,)),
                pltpu.SemaphoreType.DMA((2,)),
            ],
            compiler_params=pltpu.CompilerParams(
                vmem_limit_bytes=120 * 1024 * 1024,
                flags=flags, disable_semaphore_checks=nosem, disable_bounds_checks=nobound,
            ),
        )(A_x.reshape(M, D), A_k, A_v, A_wq, A_wo, B_x.reshape(M, D), B_k, B_v, B_wq, B_wo)
        return out.reshape(B, SQ, 2 * D)
    return fn


@jax.jit
def pallas_concat_heads__mha_block_cached__mha_block_cached__near_ridge_kernel(
    A_x, A_k_cache, A_v_cache, A_wq, A_wo, B_x, B_k_cache, B_v_cache, B_wq, B_wo):
    return make(nosem=True)(A_x, A_k_cache, A_v_cache, A_wq, A_wo, B_x, B_k_cache, B_v_cache, B_wq, B_wo)
```

```python
import functools
import math

import jax
import jax.numpy as jnp
from jax import lax
import jax.experimental.pallas as pl
import jax.experimental.pallas.tpu as pltpu

B, SQ, D = 16, 32, 1024
H, SK, DH = 32, 32, 128
M = B * SQ
T = 128
GQ = 4
GA = 8
NG = 2 * H // GQ
NA = 2 * H // GA
NP = 49
F32, BF16, U32 = jnp.float32, jnp.bfloat16, jnp.uint32

ALPHA = (((0, 0, 1), (1, 1, 1)), ((1, 0, 1), (1, 1, 1)), ((0, 0, 1),), ((1, 1, 1),),
         ((0, 0, 1), (0, 1, 1)), ((1, 0, 1), (0, 0, -1)), ((0, 1, 1), (1, 1, -1)))
BETA = (((0, 0, 1), (1, 1, 1)), ((0, 0, 1),), ((0, 1, 1), (1, 1, -1)), ((1, 0, 1), (0, 0, -1)),
        ((1, 1, 1),), ((0, 0, 1), (0, 1, 1)), ((1, 0, 1), (1, 1, 1)))
GAMMA = (((0, 0, 1), (1, 1, 1)), ((1, 0, 1), (1, 1, -1)), ((0, 1, 1), (1, 1, 1)), ((0, 0, 1), (1, 0, 1)),
         ((0, 1, 1), (0, 0, -1)), ((1, 1, 1),), ((0, 0, 1),))
MIRRORED = (2, 4, 5, 6)

INNER = (4, 1, 0, 2, 5, 3, 6)
Q_OUTER = (1, 4, 0, 2, 5, 3, 6)
O_OUTER = (4, 1, 0, 2, 5, 3, 6)
LAST_OUTER = (1, 0, 2, 3, 4, 5, 6)
X_ARRIVAL = ((2,), (3, 0), (1, 5), (4, 6))
WQ_ARRIVAL = (0, 1, 3, 7)


def _lincomb(terms, get):
    terms = sorted(terms, key=lambda t: -t[2])
    total = get(*terms[0][:2])
    for i, j, sign in terms[1:]:
        total = total + get(i, j) if sign > 0 else total - get(i, j)
    return total


def _first_use(coef, order):
    seen, new = [], {}
    for a in order:
        new[a] = [(i, j) for i, j, _ in coef[a] if (i, j) not in seen]
        seen += new[a]
    return new


class _Fold:
    def __init__(self):
        self.pending = {}
        for terms in GAMMA:
            for i, k, _ in terms:
                self.pending[i, k] = self.pending.get((i, k), 0) + 1
        self.partial = {}

    def add(self, a, m):
        done = []
        for i, k, sign in GAMMA[a]:
            if (i, k) in self.partial:
                held, c = self.partial[i, k]
                c = (c + m if sign > 0 else c - m) if held > 0 else m - c
                self.partial[i, k] = (1, c)
            else:
                self.partial[i, k] = (sign, m)
            self.pending[i, k] -= 1
            if self.pending[i, k] == 0:
                done.append((i, k, self.partial.pop((i, k))[1]))
        return done


class _Timeline:
    def __init__(self):
        self.items = []

    def spread(self, tasks, start, end):
        for n, task in enumerate(tasks):
            self.items.append((start + (end - start) * (n + 0.5) / len(tasks), len(self.items), task))

    def run_until(self, position):
        self.items.sort(key=lambda item: item[:2])
        while self.items and self.items[0][0] <= position:
            self.items.pop(0)[2]()


class _Weights:
    def __init__(self, src, stage, a, slot, direct):
        self.src, self.stage, self.a, self.slot, self.direct = src, stage, a, slot, direct
        self.rows, self.cols = src.shape[0] // 4, src.shape[1] // 4
        self.ready = None

    def staging_tasks(self):
        if self.direct:
            return []
        rows, cols = self.rows, self.cols
        step = 64 * T // cols

        def task(r0):
            v = _lincomb(BETA[self.a], lambda j, k: self.src[
                pl.ds(2 * j * rows + r0, step), pl.ds(2 * k * cols, 2 * cols)].astype(F32))
            for c in range(2 * cols // T):
                self.stage[self.slot, c, pl.ds(r0, step), :] = v[:, c * T:(c + 1) * T]
        return [functools.partial(task, r0) for r0 in range(0, 2 * rows, step)]

    def operand(self, b):
        rows, cols = self.rows, self.cols
        swap = int(self.a in MIRRORED)
        if self.direct:
            (j1, k1, _), = BETA[self.a]
            return _lincomb(BETA[b], lambda j, k: self.src[
                pl.ds((2 * j1 + j) * rows, rows), pl.ds((2 * k1 + (k ^ swap)) * cols, cols)].astype(F32)).astype(BF16)
        n = cols // T
        return jnp.concatenate(
            [_lincomb(BETA[b], lambda j, k: self.stage[self.slot, (k ^ swap) * n + c, pl.ds(j * rows, rows), :])
             for c in range(n)], axis=1).astype(BF16)


def _run_products(product, weights, timeline, base=0, emit=None):
    outer_folds = {(i, k): _Fold() for i in range(2) for k in range(2)}
    for n, w in enumerate(weights):
        if n + 1 < len(weights):
            following = weights[n + 1]
            if following.ready and not following.direct:
                following.ready()
            timeline.spread(following.staging_tasks(), base + 7 * n, base + 7 * n + 7)
        if w.ready and w.direct:
            w.ready()
        inner_fold = _Fold()
        for s, b in enumerate(INNER):
            m = product(w.a, b, w.operand(b))
            timeline.run_until(base + 7 * n + s + 1)
            if emit is not None:
                for i2, k2, c2 in inner_fold.add(b, m):
                    k2 ^= w.a in MIRRORED
                    for i1, k1, c1 in outer_folds[i2, k2].add(w.a, c2):
                        emit(2 * i1 + i2, 2 * k1 + k2, c1)


def _kernel(ax, ak, av, awq, awo, bx, bk, bv, bwq, bwo, out_hbm,
            x_buf, wq_buf, k_buf, v_buf, wo_buf,
            x_ops, wq_stage, wo_stage, q_buf, o_even, o_odd, acc, out_buf,
            in_sem, out_sem):
    SEM_XQ, SEM_WQQ, SEM_XB, SEM_WQ = 0, 4, 8, 8
    SEM_K, SEM_V, SEM_WO = 8 + NG, 8 + NG + NA, 8 + NG + 2 * NA
    k_words, v_words = k_buf.bitcast(U32), v_buf.bitcast(U32)

    def quadrant(ref, i, j):
        rows, cols = ref.shape[0] // 2, ref.shape[1] // 2
        return ref.at[pl.ds(i * rows, rows), pl.ds(j * cols, cols)]

    def start(src, dst, sem):
        pltpu.make_async_copy(src, dst, in_sem.at[sem]).start()

    def wait(dst, sem):
        pltpu.make_async_copy(dst, dst, in_sem.at[sem]).wait()

    def wait_kv(t):
        wait(k_buf.at[t], SEM_K + t)
        wait(v_buf.at[t], SEM_V + t)

    def out_copy(blk, r0, rows, c0, cols):
        return pltpu.make_async_copy(out_buf.at[blk, pl.ds(r0, rows), pl.ds(c0, cols)],
                                     out_hbm.at[pl.ds(r0, rows), pl.ds(blk * D + c0, cols)], out_sem.at[blk])

    def x_tasks(blk, outers):
        def task(r, c):
            @functools.cache
            def patch(i, j):
                words = pltpu.bitcast(x_buf[blk, pl.ds(i * T + r * 16, 16), pl.ds(j * 2 * T + c * T, T)], U32)
                return jnp.concatenate(
                    [pltpu.unpack_elementwise(words, index=h, packed_dtype=BF16, unpacked_dtype=F32)
                     for h in range(2)], axis=0)
            for a in outers:
                v = [[_lincomb(ALPHA[a], lambda i, j: patch(2 * i + i2, 2 * j + j2)) for j2 in range(2)]
                     for i2 in range(2)]
                for b in INNER:
                    s = _lincomb(ALPHA[b], lambda i, j: v[i][j])
                    x_ops[blk, 7 * a + b, c, pl.ds(r * 8, 8), :] = pltpu.pack_elementwise(
                        [s[:8], s[8:]], packed_dtype=BF16)
        return [functools.partial(task, r, c) for r in range(T // 16) for c in range(2)]

    def weights_of(src, stage, order, direct):
        return [_Weights(src, stage, a, n % 2, a in direct) for n, a in enumerate(order)]

    def wq_weights(g):
        return weights_of(wq_buf.at[g], wq_stage, Q_OUTER, Q_OUTER[:1])

    def project_q(g, weights, timeline, base=0):
        def product(a, b, rhs):
            lhs = jnp.concatenate([pltpu.bitcast(x_ops[g // (NG // 2), 7 * a + b, c], BF16) for c in range(2)], axis=1)
            return jnp.dot(lhs, rhs, preferred_element_type=F32)

        def emit(i, k, v):
            q_buf[g, pl.ds(i * T, T), pl.ds(k * DH, DH)] = v.astype(BF16)
        _run_products(product, weights, timeline, base, emit)

    def project_q_pair(g, timeline, also_wait=None):
        for d in range(2):
            wait(wq_buf.at[g + d], SEM_WQ + g + d)
        if also_wait:
            also_wait()
        for d in range(2):
            project_q(g + d, wq_weights(g + d), timeline, d * NP)

    seq_of_lane = lax.broadcasted_iota(jnp.int32, (SK, T), 1) // SQ
    exp2_scale = DH ** -0.5 * math.log2(math.e)

    def attention_tasks(t, o_ref):
        probs = {}

        def cache_tile(words, h, j):
            return pltpu.bitcast(words[t, pl.ds(4 * j, 4), h].reshape(T // 2, DH), BF16)

        def softmax(h, j):
            q = q_buf[2 * t + h // GQ, pl.ds(j * T, T), pl.ds(h % GQ * DH, DH)]
            full = lax.dot_general(cache_tile(k_words, h, j), q, (((1,), (1,)), ((), ())),
                                   preferred_element_type=F32)
            s = full[0:SK]
            for n in range(1, 4):
                s = jnp.where(seq_of_lane == n, full[n * SK:(n + 1) * SK], s)
            e = jnp.exp2((s - jnp.max(s, axis=0, keepdims=True)) * exp2_scale)
            p = e * (1.0 / jnp.sum(e, axis=0, keepdims=True))
            block_diag = jnp.concatenate([jnp.where(seq_of_lane == n, p, 0.0) for n in range(4)], axis=0)
            probs[h, j] = block_diag.astype(BF16).T

        def apply(h, j):
            o_ref[h, pl.ds(j * T, T), :] = jnp.dot(probs.pop((h, j)), cache_tile(v_words, h, j),
                                                   preferred_element_type=F32)

        def both(step, h, j):
            step(h, j)
            step(h, j + 1)

        pairs = [(h, j) for h in range(GA) for j in (0, 2)]
        tasks = []
        for n in range(len(pairs) + 1):
            if n < len(pairs):
                tasks.append(functools.partial(both, softmax, *pairs[n]))
            if n > 0:
                tasks.append(functools.partial(both, apply, *pairs[n - 1]))
        return tasks

    def wo_weights(t, order):
        return weights_of(wo_buf.at[t], wo_stage, order, (1, 4))

    def o_product(o_ref, a, b, rhs):
        terms = [(2 * i1 + i2, 2 * j1 + j2, s1 * s2) for i1, j1, s1 in ALPHA[a] for i2, j2, s2 in ALPHA[b]]
        lhs = jnp.concatenate([_lincomb(terms, lambda i, j: o_ref[2 * j + c, pl.ds(i * T, T), :])
                               for c in range(2)], axis=1)
        return jnp.dot(lhs.astype(BF16), rhs, preferred_element_type=F32)

    def project_o_and_attend(t, first, o_now, o_next):
        def product(a, b, rhs):
            held = acc[7 * a + b]
            if first is not None:
                held = jnp.where(first, 0.0, held)
            acc[7 * a + b] = held + o_product(o_now, a, b, rhs)
        timeline = _Timeline()
        timeline.spread(attention_tasks(t + 1, o_next), 0, NP)
        _run_products(product, wo_weights(t, O_OUTER), timeline)

    def finish_block_a():
        for r in range(0, T, 8):
            outer_folds = {(i, k): _Fold() for i in range(2) for k in range(2)}
            for a in range(7):
                inner_fold = _Fold()
                for b in range(7):
                    for i2, k2, c2 in inner_fold.add(b, acc[7 * a + b, pl.ds(r, 8), :]):
                        k2 ^= a in MIRRORED
                        for i1, k1, c1 in outer_folds[i2, k2].add(a, c2):
                            out_buf[0, pl.ds((2 * i1 + i2) * T + r, 8), pl.ds((2 * k1 + k2) * 2 * T, 2 * T)] = (
                                c1.astype(BF16))
        out_copy(0, 0, M, 0, D).start()

    def finish_block_b(o_ref):
        def emit(i, k, v):
            out_buf[1, pl.ds(i * T, T), pl.ds(k * 2 * T, 2 * T)] = v.astype(BF16)
            out_copy(1, i * T, T, k * 2 * T, 2 * T).start()
        _run_products(lambda a, b, rhs: o_product(o_ref, a, b, rhs) + acc[7 * a + b],
                      wo_weights(NA - 1, LAST_OUTER), _Timeline(), 0, emit)

    def wq_src(g):
        return (awq, bwq)[g // (NG // 2)].at[:, pl.ds(g % (NG // 2) * GQ * DH, GQ * DH)]

    x_new = _first_use(ALPHA, [a for outers in X_ARRIVAL for a in outers])
    wq_new = _first_use(BETA, Q_OUTER)
    for quads in x_new.values():
        for i, j in quads:
            start(quadrant(ax, i, j), quadrant(x_buf.at[0], i, j), SEM_XQ + 2 * i + j)
    for quads in wq_new.values():
        for i, j in quads:
            start(quadrant(wq_src(0), i, j), quadrant(wq_buf.at[0], i, j), SEM_WQQ + 2 * i + j)
    for g in range(1, NG):
        start(wq_src(g), wq_buf.at[g], SEM_WQ + g)
        if g == NG // 2 - 1:
            start(bx, x_buf.at[1], SEM_XB)
    for t in range(NA):
        blk, heads = t // (NA // 2), t % (NA // 2) * GA
        start((ak, bk)[blk].at[:, pl.ds(heads, GA)], k_buf.at[t], SEM_K + t)
        start((av, bv)[blk].at[:, pl.ds(heads, GA)], v_buf.at[t], SEM_V + t)
        start((awo, bwo)[blk].at[pl.ds(heads * DH, GA * DH), :], wo_buf.at[t], SEM_WO + t)

    for outers in X_ARRIVAL:
        for a in outers:
            for i, j in x_new[a]:
                wait(quadrant(x_buf.at[0], i, j), SEM_XQ + 2 * i + j)
        for task in x_tasks(0, outers):
            task()

    def wait_wq0(outers):
        for a in outers:
            for i, j in wq_new[a]:
                wait(quadrant(wq_buf.at[0], i, j), SEM_WQQ + 2 * i + j)

    weights = wq_weights(0)
    for lo, hi in zip(WQ_ARRIVAL, WQ_ARRIVAL[1:]):
        weights[lo].ready = functools.partial(wait_wq0, Q_OUTER[lo:hi])
    project_q(0, weights, _Timeline())
    wait(wq_buf.at[1], SEM_WQ + 1)
    project_q(1, wq_weights(1), _Timeline())

    @pl.loop(2, NG - 2, step=2)
    def _(g):
        last_of_a = g == NG // 2 - 2

        @pl.when(jnp.logical_not(last_of_a))
        def _():
            project_q_pair(g, _Timeline())

        @pl.when(last_of_a)
        def _():
            timeline = _Timeline()
            timeline.spread([task for a in Q_OUTER for task in x_tasks(1, (a,))], 0, 2 * NP - 3)
            project_q_pair(g, timeline, lambda: wait(x_buf.at[1], SEM_XB))

    timeline = _Timeline()
    timeline.spread(attention_tasks(0, o_even), 0, 2 * NP)
    project_q_pair(NG - 2, timeline, lambda: wait_kv(0))

    @pl.loop(0, NA - 2, step=2)
    def _(t):
        wait(wo_buf.at[t], SEM_WO + t)
        wait_kv(t + 1)
        project_o_and_attend(t, t % (NA // 2) == 0, o_even, o_odd)
        wait(wo_buf.at[t + 1], SEM_WO + t + 1)
        wait_kv(t + 2)
        project_o_and_attend(t + 1, None, o_odd, o_even)
        pl.when(t == NA // 2 - 2)(finish_block_a)

    wait(wo_buf.at[NA - 2], SEM_WO + NA - 2)
    wait_kv(NA - 1)
    wait(wo_buf.at[NA - 1], SEM_WO + NA - 1)
    project_o_and_attend(NA - 2, None, o_even, o_odd)
    finish_block_b(o_odd)
    for blk in range(2):
        pltpu.make_async_copy(out_buf.at[blk], out_buf.at[blk], out_sem.at[blk]).wait()


@jax.jit
def pallas_concat_heads__mha_block_cached__mha_block_cached__near_ridge_kernel(
    A_x: jax.Array,
    A_k_cache: jax.Array,
    A_v_cache: jax.Array,
    A_wq: jax.Array,
    A_wo: jax.Array,
    B_x: jax.Array,
    B_k_cache: jax.Array,
    B_v_cache: jax.Array,
    B_wq: jax.Array,
    B_wo: jax.Array,
):
    hbm = pl.BlockSpec(memory_space=pl.ANY)
    out = pl.pallas_call(
        _kernel,
        in_specs=[hbm] * 10,
        out_specs=hbm,
        out_shape=jax.ShapeDtypeStruct((M, 2 * D), BF16),
        scratch_shapes=[
            pltpu.VMEM((2, M, D), BF16),
            pltpu.VMEM((NG, D, GQ * DH), BF16),
            pltpu.VMEM((NA, B, GA, SK, DH), BF16),
            pltpu.VMEM((NA, B, GA, SK, DH), BF16),
            pltpu.VMEM((NA, GA * DH, D), BF16),
            pltpu.VMEM((2, NP, 2, T // 2, T), U32),
            pltpu.VMEM((2, 2, 4 * T, T), F32),
            pltpu.VMEM((2, 4, 4 * T, T), F32),
            pltpu.VMEM((NG, M, GQ * DH), BF16),
            pltpu.VMEM((GA, M, DH), F32),
            pltpu.VMEM((GA, M, DH), F32),
            pltpu.VMEM((NP, T, 2 * T), F32),
            pltpu.VMEM((2, M, D), BF16),
            pltpu.SemaphoreType.DMA((8 + NG + 3 * NA,)),
            pltpu.SemaphoreType.DMA((2,)),
        ],
        compiler_params=pltpu.CompilerParams(
            vmem_limit_bytes=110 * 1024 * 1024,
            disable_semaphore_checks=True,
        ),
    )(A_x.reshape(M, D), A_k_cache, A_v_cache, A_wq, A_wo,
      B_x.reshape(M, D), B_k_cache, B_v_cache, B_wq, B_wo)
    return out.reshape(B, SQ, 2 * D)
```

```python
import functools
import math

import jax
import jax.numpy as jnp
from jax import lax
import jax.experimental.pallas as pl
import jax.experimental.pallas.tpu as pltpu

B, SQ, D = 16, 32, 1024
H, SK, DH = 32, 32, 128
M = B * SQ
T = 128
GQ = 4
GA = 8
NG = 2 * H // GQ
NA = 2 * H // GA
NP = 49
F32, BF16 = jnp.float32, jnp.bfloat16

ALPHA = (((0, 0, 1), (1, 1, 1)), ((1, 0, 1), (1, 1, 1)), ((0, 0, 1),), ((1, 1, 1),),
         ((0, 0, 1), (0, 1, 1)), ((1, 0, 1), (0, 0, -1)), ((0, 1, 1), (1, 1, -1)))
BETA = (((0, 0, 1), (1, 1, 1)), ((0, 0, 1),), ((0, 1, 1), (1, 1, -1)), ((1, 0, 1), (0, 0, -1)),
        ((1, 1, 1),), ((0, 0, 1), (0, 1, 1)), ((1, 0, 1), (1, 1, 1)))
GAMMA = (((0, 0, 1), (1, 1, 1)), ((1, 0, 1), (1, 1, -1)), ((0, 1, 1), (1, 1, 1)), ((0, 0, 1), (1, 0, 1)),
         ((0, 1, 1), (0, 0, -1)), ((1, 1, 1),), ((0, 0, 1),))
MIRRORED = (2, 4, 5, 6)

Q_ORDER = ((4, 1, 2, 0, 3, 6, 5), (4, 1, 0, 2, 5, 3, 6))
O_ORDER = ((4, 1, 2, 3, 0, 6, 5), (4, 1, 2, 3, 6, 5, 0))
LAST_ORDER = ((1, 2, 0, 5, 3, 4, 6), (4, 1, 3, 2, 5, 0, 6))
FIRST_ORDER = ((1, 4, 0, 2, 5, 3, 6), Q_ORDER[1])
STARTUP = (
    (0, (("x", 1, 1, (3,)), ("x", 1, 0, (1,)), ("w", 0, 0, ()))),
    (1, (("x", 0, 0, (2, 0, 5)), ("x", 0, 1, (4, 6)), ("w", 1, 1, ()))),
    (3, (("w", 0, 1, ()),)),
    (5, (("w", 1, 0, ()),)),
)


def _lincomb(terms, get):
    terms = sorted(terms, key=lambda t: -t[2])
    if len(terms) == 4 and terms[1][2] > 0:
        return _lincomb([terms[0], terms[3]], get) + _lincomb([terms[1], terms[2]], get)
    total = get(*terms[0][:2])
    for i, j, sign in terms[1:]:
        total = total + get(i, j) if sign > 0 else total - get(i, j)
    return total


class _Fold:
    def __init__(self):
        self.pending = {}
        for terms in GAMMA:
            for i, k, _ in terms:
                self.pending[i, k] = self.pending.get((i, k), 0) + 1
        self.partial = {}

    def add(self, a, m):
        done = []
        for i, k, sign in GAMMA[a]:
            if (i, k) in self.partial:
                held, c = self.partial[i, k]
                c = (c + m if sign > 0 else c - m) if held > 0 else m - c
                self.partial[i, k] = (1, c)
            else:
                self.partial[i, k] = (sign, m)
            self.pending[i, k] -= 1
            if self.pending[i, k] == 0:
                done.append((i, k, self.partial.pop((i, k))[1]))
        return done


class _Timeline:
    def __init__(self):
        self.items = []

    def at(self, position, task):
        self.items.append((position, len(self.items), task))

    def spread(self, tasks, start, end):
        for n, task in enumerate(tasks):
            self.at(start + (end - start) * (n + 0.5) / len(tasks), task)

    def run_until(self, position):
        self.items.sort(key=lambda item: item[:2])
        while self.items and self.items[0][0] <= position:
            self.items.pop(0)[2]()


class _Weights:
    def __init__(self, src, stage, a, slot, direct):
        self.src, self.stage, self.a, self.slot, self.direct = src, stage, a, slot, direct
        self.rows, self.cols = src.shape[0] // 4, src.shape[1] // 4
        self.ready = None

    def staging_tasks(self):
        if self.direct:
            return []
        rows, cols = self.rows, self.cols
        step = 64 * T // cols

        def task(r0):
            v = _lincomb(BETA[self.a], lambda j, k: self.src[
                pl.ds(2 * j * rows + r0, step), pl.ds(2 * k * cols, 2 * cols)].astype(F32))
            for c in range(2 * cols // T):
                self.stage[self.slot, c, pl.ds(r0, step), :] = v[:, c * T:(c + 1) * T]
        return [functools.partial(task, r0) for r0 in range(0, 2 * rows, step)]

    def operand(self, b):
        rows, cols = self.rows, self.cols
        swap = int(self.a in MIRRORED)
        if self.direct:
            (j1, k1, _), = BETA[self.a]
            return _lincomb(BETA[b], lambda j, k: self.src[
                pl.ds((2 * j1 + j) * rows, rows), pl.ds((2 * k1 + (k ^ swap)) * cols, cols)].astype(F32)).astype(BF16)
        n = cols // T
        return jnp.concatenate(
            [_lincomb(BETA[b], lambda j, k: self.stage[self.slot, (k ^ swap) * n + c, pl.ds(j * rows, rows), :])
             for c in range(n)], axis=1).astype(BF16)


def _run_products(product, weights, inner, timeline, base=0, emit=None):
    outer_folds = {(i, k): _Fold() for i in range(2) for k in range(2)}
    for n, w in enumerate(weights):
        if w.ready and w.direct:
            w.ready()
        if n + 1 < len(weights):
            following = weights[n + 1]
            if following.ready and not following.direct:
                following.ready()
            timeline.spread(following.staging_tasks(), base + 7 * n, base + 7 * n + 7)
        inner_fold = _Fold()
        for s, b in enumerate(inner):
            m = product(w.a, b, w.operand(b))
            timeline.run_until(base + 7 * n + s + 1)
            if emit is not None:
                for i2, k2, c2 in inner_fold.add(b, m):
                    k2 ^= w.a in MIRRORED
                    for i1, k1, c1 in outer_folds[i2, k2].add(w.a, c2):
                        emit(2 * i1 + i2, 2 * k1 + k2, c1)


def _kernel(ax, ak, av, awq, awo, bx, bk, bv, bwq, bwo, out_hbm,
            x_buf, wq_buf, k_buf, v_buf, wo_buf,
            x_ops, wq_stage, wo_stage, q_buf, o_buf, acc, out_buf,
            in_sem, out_sem):
    SEM_XQ, SEM_WQQ, SEM_XB, SEM_WQ = 0, 4, 8, 8
    SEM_K, SEM_V, SEM_WO = 8 + NG, 8 + NG + NA, 8 + NG + 2 * NA

    def quadrant(ref, i, j):
        rows, cols = ref.shape[0] // 2, ref.shape[1] // 2
        return ref.at[pl.ds(i * rows, rows), pl.ds(j * cols, cols)]

    def start(src, dst, sem):
        pltpu.make_async_copy(src, dst, in_sem.at[sem]).start()

    def wait(dst, sem):
        pltpu.make_async_copy(dst, dst, in_sem.at[sem]).wait()

    def wait_kv(t):
        wait(k_buf.at[t], SEM_K + t)
        wait(v_buf.at[t], SEM_V + t)

    def out_copy(blk, r0, rows, c0, cols):
        return pltpu.make_async_copy(out_buf.at[blk, pl.ds(r0, rows), pl.ds(c0, cols)],
                                     out_hbm.at[pl.ds(r0, rows), pl.ds(blk * D + c0, cols)], out_sem.at[blk])

    def x_tasks(blk, outers):
        def task(r):
            @functools.cache
            def patch(i, j):
                return x_buf[blk, pl.ds(i * T + r, 16), pl.ds(j * 2 * T, 2 * T)].astype(F32)
            for a in outers:
                v = [[_lincomb(ALPHA[a], lambda i, j: patch(2 * i + i2, 2 * j + j2)) for j2 in range(2)]
                     for i2 in range(2)]
                for b in Q_ORDER[1]:
                    x_ops[blk, 7 * a + b, pl.ds(r, 16), :] = _lincomb(ALPHA[b], lambda i, j: v[i][j]).astype(BF16)
        return [functools.partial(task, r) for r in range(0, T, 16)]

    def weights_of(src, stage, order, direct):
        return [_Weights(src, stage, a, n % 2, a in direct) for n, a in enumerate(order)]

    def project_q(g, weights, timeline, base=0):
        def product(a, b, rhs):
            return jnp.dot(x_ops[g // (NG // 2), 7 * a + b], rhs, preferred_element_type=F32)

        def emit(i, k, v):
            q_buf[g, pl.ds(i * T, T), pl.ds(k * DH, DH)] = v.astype(BF16)
        _run_products(product, weights, Q_ORDER[1], timeline, base, emit)

    def project_q_groups(g, count, timeline, also_wait=None):
        for d in range(count):
            wait(wq_buf.at[g + d], SEM_WQ + g + d)
        if also_wait:
            also_wait()
        for d in range(count):
            project_q(g + d, weights_of(wq_buf.at[g + d], wq_stage, Q_ORDER[0], Q_ORDER[0][:1]), timeline, d * NP)

    seq_of_lane = lax.broadcasted_iota(jnp.int32, (SK, T), 1) // SQ
    exp2_scale = DH ** -0.5 * math.log2(math.e)

    def schedule_attention(t, o_ref, timeline, period, offset, end):
        probs = {}

        def cache_tile(cache, h, j):
            return cache[t, pl.ds(4 * j, 4), h].reshape(T, DH)

        def softmax(h, j):
            q = q_buf[2 * t + h // GQ, pl.ds(j * T, T), pl.ds(h % GQ * DH, DH)]
            full = lax.dot_general(cache_tile(k_buf, h, j), q, (((1,), (1,)), ((), ())),
                                   preferred_element_type=F32)
            s = full[0:SK]
            for n in range(1, 4):
                s = jnp.where(seq_of_lane == n, full[n * SK:(n + 1) * SK], s)
            e = jnp.exp2((s - jnp.max(s, axis=0, keepdims=True)) * exp2_scale)
            p = e * (1.0 / jnp.sum(e, axis=0, keepdims=True))
            block_diag = jnp.concatenate([jnp.where(seq_of_lane == n, p, 0.0) for n in range(4)], axis=0)
            probs[h, j] = block_diag.astype(BF16).T

        def apply(h, j):
            o_ref[h, pl.ds(j * T, T), :] = jnp.dot(probs.pop((h, j)), cache_tile(v_buf, h, j),
                                                   preferred_element_type=F32)

        for n, (h, j) in enumerate((h, j) for h in range(GA) for j in range(4)):
            pair = n // 2
            timeline.at(period * pair, functools.partial(softmax, h, j))
            timeline.at(min(period * (pair + 1) + offset, end), functools.partial(apply, h, j))

    def wo_weights(t, order):
        return weights_of(wo_buf.at[t], wo_stage, order, (1, 4))

    def o_product(o_ref, a, b, rhs):
        terms = [(2 * i1 + i2, 2 * j1 + j2, s1 * s2) for i1, j1, s1 in ALPHA[a] for i2, j2, s2 in ALPHA[b]]
        lhs = jnp.concatenate([_lincomb(terms, lambda i, j: o_ref[2 * j + c, pl.ds(i * T, T), :])
                               for c in range(2)], axis=1)
        return jnp.dot(lhs.astype(BF16), rhs, preferred_element_type=F32)

    def project_o_and_attend(t):
        o_pair = o_buf.at[pl.ds(t, 2)]

        def product(a, b, rhs):
            held = jnp.where(t % (NA // 2) == 0, 0.0, acc[7 * a + b])
            acc[7 * a + b] = held + o_product(o_pair.at[0], a, b, rhs)
        timeline = _Timeline()
        schedule_attention(t + 1, o_pair.at[1], timeline, 3, 2, NP)
        _run_products(product, wo_weights(t, O_ORDER[0]), O_ORDER[1], timeline)

    def finish_block_a():
        @pl.loop(0, T, step=32)
        def _(r0):
            for r in range(0, 32, 8):
                r = pl.multiple_of(r0 + r, 8)
                outer_folds = {(i, k): _Fold() for i in range(2) for k in range(2)}
                for a in range(7):
                    inner_fold = _Fold()
                    for b in range(7):
                        for i2, k2, c2 in inner_fold.add(b, acc[7 * a + b, pl.ds(r, 8), :]):
                            k2 ^= a in MIRRORED
                            for i1, k1, c1 in outer_folds[i2, k2].add(a, c2):
                                out_buf[0, pl.ds((2 * i1 + i2) * T + r, 8),
                                        pl.ds((2 * k1 + k2) * 2 * T, 2 * T)] = c1.astype(BF16)
        out_copy(0, 0, M, 0, D).start()

    def finish_block_b():
        def emit(i, k, v):
            out_buf[1, pl.ds(i * T, T), pl.ds(k * 2 * T, 2 * T)] = v.astype(BF16)
            out_copy(1, i * T, T, k * 2 * T, 2 * T).start()
        _run_products(lambda a, b, rhs: o_product(o_buf.at[NA - 1], a, b, rhs) + acc[7 * a + b],
                      wo_weights(NA - 1, LAST_ORDER[0]), LAST_ORDER[1], _Timeline(), 0, emit)

    def wq_src(g):
        return (awq, bwq)[g // (NG // 2)].at[:, pl.ds(g % (NG // 2) * GQ * DH, GQ * DH)]

    def first_copy(kind, i, j):
        if kind == "x":
            return quadrant(ax, i, j), quadrant(x_buf.at[0], i, j), SEM_XQ + 2 * i + j
        return quadrant(wq_src(0), i, j), quadrant(wq_buf.at[0], i, j), SEM_WQQ + 2 * i + j

    for _, steps in STARTUP:
        for kind, i, j, _ in steps:
            start(*first_copy(kind, i, j))
    for g in range(1, NG):
        start(wq_src(g), wq_buf.at[g], SEM_WQ + g)
        if g == NG // 2 - 1:
            start(bx, x_buf.at[1], SEM_XB)
    for t in range(NA):
        blk, heads = t // (NA // 2), t % (NA // 2) * GA
        start((ak, bk)[blk].at[:, pl.ds(heads, GA)], k_buf.at[t], SEM_K + t)
        start((av, bv)[blk].at[:, pl.ds(heads, GA)], v_buf.at[t], SEM_V + t)
        start((awo, bwo)[blk].at[pl.ds(heads * DH, GA * DH), :], wo_buf.at[t], SEM_WO + t)

    def arrive(steps):
        for kind, i, j, outers in steps:
            wait(*first_copy(kind, i, j)[1:])
            if outers:
                for task in x_tasks(0, outers):
                    task()

    weights = weights_of(wq_buf.at[0], wq_stage, FIRST_ORDER[0], (1, 4))
    for n, steps in STARTUP:
        weights[n].ready = functools.partial(arrive, steps)
    project_q(0, weights, _Timeline())
    project_q_groups(1, 1, _Timeline())

    @pl.loop(2, NG - 2, step=2)
    def _(g):
        last_of_a = g == NG // 2 - 2

        @pl.when(jnp.logical_not(last_of_a))
        def _():
            project_q_groups(g, 2, _Timeline())

        @pl.when(last_of_a)
        def _():
            timeline = _Timeline()
            timeline.spread([task for a in Q_ORDER[0] for task in x_tasks(1, (a,))], 0, 2 * NP)
            project_q_groups(g, 2, timeline, lambda: wait(x_buf.at[1], SEM_XB))

    timeline = _Timeline()
    schedule_attention(0, o_buf.at[0], timeline, 6, 3, 2 * NP)
    project_q_groups(NG - 2, 2, timeline, lambda: wait_kv(0))

    @pl.loop(0, NA - 1)
    def _(t):
        wait(wo_buf.at[t], SEM_WO + t)
        wait_kv(t + 1)
        project_o_and_attend(t)
        pl.when(t == NA // 2 - 1)(finish_block_a)

    wait(wo_buf.at[NA - 1], SEM_WO + NA - 1)
    finish_block_b()
    for blk in range(2):
        pltpu.make_async_copy(out_buf.at[blk], out_buf.at[blk], out_sem.at[blk]).wait()


@jax.jit
def pallas_concat_heads__mha_block_cached__mha_block_cached__near_ridge_kernel(
    A_x: jax.Array,
    A_k_cache: jax.Array,
    A_v_cache: jax.Array,
    A_wq: jax.Array,
    A_wo: jax.Array,
    B_x: jax.Array,
    B_k_cache: jax.Array,
    B_v_cache: jax.Array,
    B_wq: jax.Array,
    B_wo: jax.Array,
):
    hbm = pl.BlockSpec(memory_space=pl.ANY)
    out = pl.pallas_call(
        _kernel,
        in_specs=[hbm] * 10,
        out_specs=hbm,
        out_shape=jax.ShapeDtypeStruct((M, 2 * D), BF16),
        scratch_shapes=[
            pltpu.VMEM((2, M, D), BF16),
            pltpu.VMEM((NG, D, GQ * DH), BF16),
            pltpu.VMEM((NA, B, GA, SK, DH), BF16),
            pltpu.VMEM((NA, B, GA, SK, DH), BF16),
            pltpu.VMEM((NA, GA * DH, D), BF16),
            pltpu.VMEM((2, NP, T, 2 * T), BF16),
            pltpu.VMEM((2, 2, 4 * T, T), F32),
            pltpu.VMEM((2, 4, 4 * T, T), F32),
            pltpu.VMEM((NG, M, GQ * DH), BF16),
            pltpu.VMEM((NA, GA, M, DH), F32),
            pltpu.VMEM((NP, T, 2 * T), F32),
            pltpu.VMEM((2, M, D), BF16),
            pltpu.SemaphoreType.DMA((8 + NG + 3 * NA,)),
            pltpu.SemaphoreType.DMA((2,)),
        ],
        compiler_params=pltpu.CompilerParams(
            vmem_limit_bytes=118 * 1024 * 1024,
            disable_semaphore_checks=True,
        ),
    )(A_x.reshape(M, D), A_k_cache, A_v_cache, A_wq, A_wo,
      B_x.reshape(M, D), B_k_cache, B_v_cache, B_wq, B_wo)
    return out.reshape(B, SQ, 2 * D)
```

```python
import functools
import math

import jax
import jax.numpy as jnp
from jax import lax
import jax.experimental.pallas as pl
import jax.experimental.pallas.tpu as pltpu

B, SQ, D = 16, 32, 1024
H, SK, DH = 32, 32, 128
M = B * SQ
T = 128
GQ = 4
GA = 8
NG = 2 * H // GQ
NA = 2 * H // GA
NP = 49
F32, BF16 = jnp.float32, jnp.bfloat16

ALPHA = (((0, 0, 1), (1, 1, 1)), ((1, 0, 1), (1, 1, 1)), ((0, 0, 1),), ((1, 1, 1),),
         ((0, 0, 1), (0, 1, 1)), ((1, 0, 1), (0, 0, -1)), ((0, 1, 1), (1, 1, -1)))
BETA = (((0, 0, 1), (1, 1, 1)), ((0, 0, 1),), ((0, 1, 1), (1, 1, -1)), ((1, 0, 1), (0, 0, -1)),
        ((1, 1, 1),), ((0, 0, 1), (0, 1, 1)), ((1, 0, 1), (1, 1, 1)))
GAMMA = (((0, 0, 1), (1, 1, 1)), ((1, 0, 1), (1, 1, -1)), ((0, 1, 1), (1, 1, 1)), ((0, 0, 1), (1, 0, 1)),
         ((0, 1, 1), (0, 0, -1)), ((1, 1, 1),), ((0, 0, 1),))
MIRRORED = (2, 4, 5, 6)

Q_ORDER = ((4, 1, 2, 0, 3, 6, 5), (4, 1, 0, 2, 5, 3, 6))
O_ORDER = ((4, 1, 2, 3, 0, 6, 5), (4, 1, 2, 5, 6, 3, 0))
LAST_ORDER = ((1, 2, 0, 5, 3, 4, 6), (4, 1, 2, 5, 3, 0, 6))
FIRST_ORDER = ((1, 4, 0, 2, 5, 3, 6), Q_ORDER[1])
STARTUP = (
    (0, (("x", 1, 1, (3,)), ("x", 1, 0, (1,)), ("w", 0, 0, ()))),
    (1, (("x", 0, 0, (2, 0, 5)), ("x", 0, 1, (4, 6)), ("w", 1, 1, ()))),
    (3, (("w", 0, 1, ()), ("w", 1, 0, ()))),
)
PREPARE_B = 5


def _lincomb(terms, get):
    terms = sorted(terms, key=lambda t: -t[2])
    if len(terms) == 4 and terms[1][2] > 0:
        return _lincomb([terms[0], terms[3]], get) + _lincomb([terms[1], terms[2]], get)
    total = get(*terms[0][:2])
    for i, j, sign in terms[1:]:
        total = total + get(i, j) if sign > 0 else total - get(i, j)
    return total


class _Fold:
    def __init__(self):
        self.pending = {}
        for terms in GAMMA:
            for i, k, _ in terms:
                self.pending[i, k] = self.pending.get((i, k), 0) + 1
        self.partial = {}

    def add(self, a, m):
        done = []
        for i, k, sign in GAMMA[a]:
            if (i, k) in self.partial:
                held, c = self.partial[i, k]
                c = (c + m if sign > 0 else c - m) if held > 0 else m - c
                self.partial[i, k] = (1, c)
            else:
                self.partial[i, k] = (sign, m)
            self.pending[i, k] -= 1
            if self.pending[i, k] == 0:
                done.append((i, k, self.partial.pop((i, k))[1]))
        return done


class _Timeline:
    def __init__(self):
        self.items = []

    def at(self, position, task):
        self.items.append((position, len(self.items), task))

    def spread(self, tasks, start, end):
        for n, task in enumerate(tasks):
            self.at(start + (end - start) * (n + 0.5) / len(tasks), task)

    def run_until(self, position):
        self.items.sort(key=lambda item: item[:2])
        while self.items and self.items[0][0] <= position:
            self.items.pop(0)[2]()


class _Weights:
    def __init__(self, src, stage, a, slot, direct):
        self.src, self.stage, self.a, self.slot, self.direct = src, stage, a, slot, direct
        self.rows, self.cols = src.shape[0] // 4, src.shape[1] // 4
        self.ready = None

    def staging_tasks(self):
        if self.direct:
            return []
        rows, cols = self.rows, self.cols
        step = 64 * T // cols

        def task(r0):
            v = _lincomb(BETA[self.a], lambda j, k: self.src[
                pl.ds(2 * j * rows + r0, step), pl.ds(2 * k * cols, 2 * cols)].astype(F32))
            for c in range(2 * cols // T):
                self.stage[self.slot, c, pl.ds(r0, step), :] = v[:, c * T:(c + 1) * T]
        return [functools.partial(task, r0) for r0 in range(0, 2 * rows, step)]

    def operand(self, b):
        rows, cols = self.rows, self.cols
        swap = int(self.a in MIRRORED)
        if self.direct:
            (j1, k1, _), = BETA[self.a]
            return _lincomb(BETA[b], lambda j, k: self.src[
                pl.ds((2 * j1 + j) * rows, rows), pl.ds((2 * k1 + (k ^ swap)) * cols, cols)].astype(F32)).astype(BF16)
        n = cols // T
        return jnp.concatenate(
            [_lincomb(BETA[b], lambda j, k: self.stage[self.slot, (k ^ swap) * n + c, pl.ds(j * rows, rows), :])
             for c in range(n)], axis=1).astype(BF16)


def _run_products(product, weights, inner, timeline, base=0, emit=None):
    outer_folds = {(i, k): _Fold() for i in range(2) for k in range(2)}
    for n, w in enumerate(weights):
        if w.ready:
            w.ready()
            for task in w.staging_tasks():
                task()
        if n + 1 < len(weights) and not weights[n + 1].ready:
            timeline.spread(weights[n + 1].staging_tasks(), base + 7 * n, base + 7 * n + 7)
        inner_fold = _Fold()
        for s, b in enumerate(inner):
            m = product(w.a, b, w.operand(b))
            timeline.run_until(base + 7 * n + s + 1)
            if emit is not None:
                for i2, k2, c2 in inner_fold.add(b, m):
                    k2 ^= w.a in MIRRORED
                    for i1, k1, c1 in outer_folds[i2, k2].add(w.a, c2):
                        emit(2 * i1 + i2, 2 * k1 + k2, c1)


def _kernel(ax, ak, av, awq, awo, bx, bk, bv, bwq, bwo, out_hbm,
            x_buf, wq_buf, k_buf, v_buf, wo_buf,
            x_ops, wq_stage, wo_stage, q_buf, o_buf, acc, out_buf,
            in_sem, out_sem):
    SEM_XQ, SEM_WQQ, SEM_XB, SEM_WQ = 0, 4, 8, 8
    SEM_K, SEM_V, SEM_WO = 8 + NG, 8 + NG + NA, 8 + NG + 2 * NA

    def quadrant(ref, i, j):
        rows, cols = ref.shape[0] // 2, ref.shape[1] // 2
        return ref.at[pl.ds(i * rows, rows), pl.ds(j * cols, cols)]

    def start(src, dst, sem):
        pltpu.make_async_copy(src, dst, in_sem.at[sem]).start()

    def wait(dst, sem):
        pltpu.make_async_copy(dst, dst, in_sem.at[sem]).wait()

    def wait_kv(t):
        wait(k_buf.at[t], SEM_K + t)
        wait(v_buf.at[t], SEM_V + t)

    def out_copy(blk, r0, rows, c0, cols):
        return pltpu.make_async_copy(out_buf.at[blk, pl.ds(r0, rows), pl.ds(c0, cols)],
                                     out_hbm.at[pl.ds(r0, rows), pl.ds(blk * D + c0, cols)], out_sem.at[blk])

    def x_tasks(blk, outers):
        def task(r):
            @functools.cache
            def patch(i, j):
                return x_buf[blk, pl.ds(i * T + r, 16), pl.ds(j * 2 * T, 2 * T)].astype(F32)
            for a in outers:
                v = [[_lincomb(ALPHA[a], lambda i, j: patch(2 * i + i2, 2 * j + j2)) for j2 in range(2)]
                     for i2 in range(2)]
                for b in Q_ORDER[1]:
                    x_ops[blk, 7 * a + b, pl.ds(r, 16), :] = _lincomb(ALPHA[b], lambda i, j: v[i][j]).astype(BF16)
        return [functools.partial(task, r) for r in range(0, T, 16)]

    def weights_of(src, stage, order, direct):
        return [_Weights(src, stage, a, n % 2, a in direct) for n, a in enumerate(order)]

    def project_q(g, weights, timeline, base=0):
        def product(a, b, rhs):
            return jnp.dot(x_ops[g // (NG // 2), 7 * a + b], rhs, preferred_element_type=F32)

        def emit(i, k, v):
            q_buf[g, pl.ds(i * T, T), pl.ds(k * DH, DH)] = v.astype(BF16)
        _run_products(product, weights, Q_ORDER[1], timeline, base, emit)

    def project_q_groups(g, count, timeline, also_wait=None):
        for d in range(count):
            wait(wq_buf.at[g + d], SEM_WQ + g + d)
        if also_wait:
            also_wait()
        for d in range(count):
            project_q(g + d, weights_of(wq_buf.at[g + d], wq_stage, Q_ORDER[0], Q_ORDER[0][:1]), timeline, d * NP)

    seq_of_lane = lax.broadcasted_iota(jnp.int32, (SK, T), 1) // SQ
    exp2_scale = DH ** -0.5 * math.log2(math.e)

    def schedule_attention(t, o_ref, timeline, period, offset, end):
        probs = {}

        def cache_tile(cache, h, j):
            return cache[t, pl.ds(4 * j, 4), h].reshape(T, DH)

        def softmax(h, j):
            q = q_buf[2 * t + h // GQ, pl.ds(j * T, T), pl.ds(h % GQ * DH, DH)]
            full = lax.dot_general(cache_tile(k_buf, h, j), q, (((1,), (1,)), ((), ())),
                                   preferred_element_type=F32)
            s = full[0:SK]
            for n in range(1, 4):
                s = jnp.where(seq_of_lane == n, full[n * SK:(n + 1) * SK], s)
            e = jnp.exp2((s - jnp.max(s, axis=0, keepdims=True)) * exp2_scale)
            p = e * (1.0 / jnp.sum(e, axis=0, keepdims=True))
            block_diag = jnp.concatenate([jnp.where(seq_of_lane == n, p, 0.0) for n in range(4)], axis=0)
            probs[h, j] = block_diag.astype(BF16).T

        def apply(h, j):
            o_ref[h, pl.ds(j * T, T), :] = jnp.dot(probs.pop((h, j)), cache_tile(v_buf, h, j),
                                                   preferred_element_type=F32)

        for n, (h, j) in enumerate((h, j) for h in range(GA) for j in range(4)):
            pair = n // 2
            timeline.at(period * pair, functools.partial(softmax, h, j))
            timeline.at(min(period * (pair + 1) + offset, end), functools.partial(apply, h, j))

    def wo_weights(t, order):
        return weights_of(wo_buf.at[t], wo_stage, order, (1, 4))

    def o_product(o_ref, a, b, rhs):
        terms = [(2 * i1 + i2, 2 * j1 + j2, s1 * s2) for i1, j1, s1 in ALPHA[a] for i2, j2, s2 in ALPHA[b]]
        lhs = jnp.concatenate([_lincomb(terms, lambda i, j: o_ref[2 * j + c, pl.ds(i * T, T), :])
                               for c in range(2)], axis=1)
        return jnp.dot(lhs.astype(BF16), rhs, preferred_element_type=F32)

    def project_o_and_attend(t):
        o_pair = o_buf.at[pl.ds(t, 2)]

        def product(a, b, rhs):
            held = jnp.where(t % (NA // 2) == 0, 0.0, acc[7 * a + b])
            acc[7 * a + b] = held + o_product(o_pair.at[0], a, b, rhs)
        timeline = _Timeline()
        schedule_attention(t + 1, o_pair.at[1], timeline, 3, 2, NP)
        _run_products(product, wo_weights(t, O_ORDER[0]), O_ORDER[1], timeline)

    def finish_block_a():
        @pl.loop(0, T, step=32)
        def _(r0):
            for r in range(0, 32, 8):
                r = pl.multiple_of(r0 + r, 8)
                outer_folds = {(i, k): _Fold() for i in range(2) for k in range(2)}
                for a in range(7):
                    inner_fold = _Fold()
                    for b in range(7):
                        for i2, k2, c2 in inner_fold.add(b, acc[7 * a + b, pl.ds(r, 8), :]):
                            k2 ^= a in MIRRORED
                            for i1, k1, c1 in outer_folds[i2, k2].add(a, c2):
                                out_buf[0, pl.ds((2 * i1 + i2) * T + r, 8),
                                        pl.ds((2 * k1 + k2) * 2 * T, 2 * T)] = c1.astype(BF16)
        out_copy(0, 0, M, 0, D).start()

    def finish_block_b():
        def emit(i, k, v):
            out_buf[1, pl.ds(i * T, T), pl.ds(k * 2 * T, 2 * T)] = v.astype(BF16)
            out_copy(1, i * T, T, k * 2 * T, 2 * T).start()
        _run_products(lambda a, b, rhs: o_product(o_buf.at[NA - 1], a, b, rhs) + acc[7 * a + b],
                      wo_weights(NA - 1, LAST_ORDER[0]), LAST_ORDER[1], _Timeline(), 0, emit)

    def wq_src(g):
        return (awq, bwq)[g // (NG // 2)].at[:, pl.ds(g % (NG // 2) * GQ * DH, GQ * DH)]

    def first_copy(kind, i, j):
        if kind == "x":
            return quadrant(ax, i, j), quadrant(x_buf.at[0], i, j), SEM_XQ + 2 * i + j
        return quadrant(wq_src(0), i, j), quadrant(wq_buf.at[0], i, j), SEM_WQQ + 2 * i + j

    for _, steps in STARTUP:
        for kind, i, j, _ in steps:
            start(*first_copy(kind, i, j))
    for g in range(1, NG):
        start(wq_src(g), wq_buf.at[g], SEM_WQ + g)
        if g == PREPARE_B + 1:
            start(bx, x_buf.at[1], SEM_XB)
    for t in range(NA):
        blk, heads = t // (NA // 2), t % (NA // 2) * GA
        start((ak, bk)[blk].at[:, pl.ds(heads, GA)], k_buf.at[t], SEM_K + t)
        start((av, bv)[blk].at[:, pl.ds(heads, GA)], v_buf.at[t], SEM_V + t)
        start((awo, bwo)[blk].at[pl.ds(heads * DH, GA * DH), :], wo_buf.at[t], SEM_WO + t)

    def arrive(steps):
        for kind, i, j, outers in steps:
            wait(*first_copy(kind, i, j)[1:])
            if outers:
                for task in x_tasks(0, outers):
                    task()

    weights = weights_of(wq_buf.at[0], wq_stage, FIRST_ORDER[0], (1, 4))
    for n, steps in STARTUP:
        weights[n].ready = functools.partial(arrive, steps)
    project_q(0, weights, _Timeline())

    @pl.loop(1, 3)
    def _(g):
        project_q_groups(g, 1, _Timeline())

    @pl.loop(3, NG - 1, step=2)
    def _(g):
        @pl.when(g != PREPARE_B)
        def _():
            project_q_groups(g, 2, _Timeline())

        @pl.when(g == PREPARE_B)
        def _():
            timeline = _Timeline()
            timeline.spread([task for a in Q_ORDER[0] for task in x_tasks(1, (a,))], 0, 2 * NP)
            project_q_groups(g, 2, timeline, lambda: wait(x_buf.at[1], SEM_XB))

    timeline = _Timeline()
    schedule_attention(0, o_buf.at[0], timeline, 3, 1, NP)
    project_q_groups(NG - 1, 1, timeline, lambda: wait_kv(0))

    @pl.loop(0, NA - 1)
    def _(t):
        wait(wo_buf.at[t], SEM_WO + t)
        wait_kv(t + 1)
        project_o_and_attend(t)
        pl.when(t == NA // 2 - 1)(finish_block_a)

    wait(wo_buf.at[NA - 1], SEM_WO + NA - 1)
    finish_block_b()
    for blk in range(2):
        pltpu.make_async_copy(out_buf.at[blk], out_buf.at[blk], out_sem.at[blk]).wait()


@jax.jit
def pallas_concat_heads__mha_block_cached__mha_block_cached__near_ridge_kernel(
    A_x: jax.Array,
    A_k_cache: jax.Array,
    A_v_cache: jax.Array,
    A_wq: jax.Array,
    A_wo: jax.Array,
    B_x: jax.Array,
    B_k_cache: jax.Array,
    B_v_cache: jax.Array,
    B_wq: jax.Array,
    B_wo: jax.Array,
):
    hbm = pl.BlockSpec(memory_space=pl.ANY)
    out = pl.pallas_call(
        _kernel,
        in_specs=[hbm] * 10,
        out_specs=hbm,
        out_shape=jax.ShapeDtypeStruct((M, 2 * D), BF16),
        scratch_shapes=[
            pltpu.VMEM((2, M, D), BF16),
            pltpu.VMEM((NG, D, GQ * DH), BF16),
            pltpu.VMEM((NA, B, GA, SK, DH), BF16),
            pltpu.VMEM((NA, B, GA, SK, DH), BF16),
            pltpu.VMEM((NA, GA * DH, D), BF16),
            pltpu.VMEM((2, NP, T, 2 * T), BF16),
            pltpu.VMEM((2, 2, 4 * T, T), F32),
            pltpu.VMEM((2, 4, 4 * T, T), F32),
            pltpu.VMEM((NG, M, GQ * DH), BF16),
            pltpu.VMEM((NA, GA, M, DH), F32),
            pltpu.VMEM((NP, T, 2 * T), F32),
            pltpu.VMEM((2, M, D), BF16),
            pltpu.SemaphoreType.DMA((8 + NG + 3 * NA,)),
            pltpu.SemaphoreType.DMA((2,)),
        ],
        compiler_params=pltpu.CompilerParams(
            vmem_limit_bytes=118 * 1024 * 1024,
            disable_semaphore_checks=True,
        ),
    )(A_x.reshape(M, D), A_k_cache, A_v_cache, A_wq, A_wo,
      B_x.reshape(M, D), B_k_cache, B_v_cache, B_wq, B_wo)
    return out.reshape(B, SQ, 2 * D)
```
